```python
import jax
import jax.numpy as jnp

def _softmax(x, axis=-1):
    return jax.nn.softmax(x, axis=axis)

def _gelu(x):
    return jax.nn.gelu(x, approximate=True)

def _silu(x):
    return jax.nn.silu(x)

def _sigmoid(x):
    return jax.nn.sigmoid(x)

def _layernorm(x, axis=-1, eps=1e-05):
    m = jnp.mean(x, axis=axis, keepdims=True)
    v = jnp.var(x, axis=axis, keepdims=True)
    return (x - m) / jnp.sqrt(v + eps)

def _scatter_add(tgt, idx, src, axis=0):
    return tgt.at[idx].add(src)

def _segment_sum(src, seg, n):
    return jax.ops.segment_sum(src, seg, n)

class _Rng:

    def __init__(self, key):
        self._k = key

    def _next(self):
        self._k, sub = jax.random.split(self._k)
        return sub

    def normal(self, shape):
        return jax.random.normal(self._next(), shape, dtype=jnp.bfloat16)

    def randint(self, lo, hi, shape):
        return jax.random.randint(self._next(), shape, lo, hi, dtype=jnp.int32)

    def uniform(self, shape, lo=0.0, hi=1.0):
        return jax.random.uniform(self._next(), shape, jnp.bfloat16, lo, hi)

    def permutation(self, n):
        return jax.random.permutation(self._next(), n)
kernel_name = 'adaLN_cond__compressed_kv_cla__glu_gated_geglu__decode'

def setup_inputs():
    _rng = _Rng(jax.random.key(int.from_bytes(__import__("os").urandom(4), "little")))
    _w = lambda a: (lambda t: t.astype(jnp.bfloat16) if jnp.issubdtype(t.dtype, jnp.floating) else t)(jnp.asarray(a))

    def _A_setup():
        B, H, Sq, Sk, D, M = (1, 32, 1, 32768, 128, 512)
        Dc = 4 * D
        return {'x': _w((lambda *s: _rng.normal(s) * 0.05)(B, Sq, M)), 'c_kv': _w((lambda *s: _rng.normal(s) * 0.05)(B, Sk, Dc)), 'w_q': _w((lambda *s: _rng.normal(s) * 0.05)(M, H, D) * M ** (-0.5)), 'w_uk': _w((lambda *s: _rng.normal(s) * 0.05)(Dc, H, D) * Dc ** (-0.5)), 'w_uv': _w((lambda *s: _rng.normal(s) * 0.05)(Dc, H, D) * Dc ** (-0.5)), 'w_o': _w((lambda *s: _rng.normal(s) * 0.05)(H, D, M) * (H * D) ** (-0.5))}
    _A_in = _A_setup()

    def _B_setup():
        B, S, Dm, Df = (1, 1, 512, 1792)
        return {'x': _w((lambda *s: _rng.normal(s) * 0.05)(B, S, Dm)), 'w_gate': _w((lambda *s: _rng.normal(s) * 0.05)(Dm, Df) * Dm ** (-0.5)), 'w_up': _w((lambda *s: _rng.normal(s) * 0.05)(Dm, Df) * Dm ** (-0.5)), 'w_down': _w((lambda *s: _rng.normal(s) * 0.05)(Df, Dm) * Df ** (-0.5))}
    _B_in = _B_setup()
    return {'A_x': _A_in['x'], 'A_c_kv': _A_in['c_kv'], 'A_w_q': _A_in['w_q'], 'A_w_uk': _A_in['w_uk'], 'A_w_uv': _A_in['w_uv'], 'A_w_o': _A_in['w_o'], 'B_x': _B_in['x'], 'B_w_gate': _B_in['w_gate'], 'B_w_up': _B_in['w_up'], 'B_w_down': _B_in['w_down'], 'c': _w((lambda *s: _rng.normal(s) * 0.05)(1, 512)), 'w_mod': _w((lambda *s: _rng.normal(s) * 0.05)(512, 6 * 512) * 512 ** (-0.5))}

def reference(A_x, A_c_kv, A_w_q, A_w_uk, A_w_uv, A_w_o, B_x, B_w_gate, B_w_up, B_w_down, c, w_mod):

    def _A_ref(x, c_kv, w_q, w_uk, w_uv, w_o):
        B, Sq, M = (x.shape[0], x.shape[1], x.shape[2])
        Sk = c_kv.shape[1]
        H, D = (w_q.shape[1], w_q.shape[2])
        q = jnp.einsum('bqm,mhd->bhqd', x, w_q)
        k = jnp.einsum('bkc,chd->bhkd', c_kv, w_uk)
        v = jnp.einsum('bkc,chd->bhkd', c_kv, w_uv)
        scores = jnp.einsum('bhqd,bhkd->bhqk', q, k) * D ** (-0.5)
        off = Sk - Sq
        qi = jnp.arange(Sq)[:, None]
        kj = jnp.arange(Sk)[None, :]
        cmask = kj <= qi + off
        scores = jnp.where(cmask[None, None], scores, -1000000000.0)
        p = _softmax(scores, axis=-1)
        ctx = jnp.einsum('bhqk,bhkd->bhqd', p, v)
        return jnp.einsum('bhqd,hdm->bqm', ctx, w_o)

    def _B_ref(x, w_gate, w_up, w_down):
        g = jnp.einsum('bsd,df->bsf', x, w_gate)
        u = jnp.einsum('bsd,df->bsf', x, w_up)
        h = _gelu(g) * u
        return jnp.einsum('bsf,fd->bsd', h, w_down)
    x = A_x
    mod = (_silu(c) @ w_mod).reshape(c.shape[0], 6, 1, -1)
    sa, ca, ga, sb, cb, gb = (mod[:, 0].copy(), mod[:, 1].copy(), mod[:, 2].copy(), mod[:, 3].copy(), mod[:, 4].copy(), mod[:, 5].copy())
    h = _layernorm(x, axis=-1) * (1 + ca) + sa
    x = x + ga * _A_ref(h, A_c_kv, A_w_q, A_w_uk, A_w_uv, A_w_o)
    h = _layernorm(x, axis=-1) * (1 + cb) + sb
    x = x + gb * _B_ref(h, B_w_gate, B_w_up, B_w_down)
    return x
```

```python
import functools

import jax
import jax.numpy as jnp
import jax.experimental.pallas as pl
import jax.experimental.pallas.tpu as pltpu

_F32 = jnp.float32
_BF16 = jnp.bfloat16
_NN = (((1,), (0,)), ((), ()))
_NT = (((1,), (1,)), ((), ()))

_KV_CHUNK = 4096
_KV_TILE = 2048
_DOWN_TAIL = 256
_LANES = 128


def _dot(a, b, dims=_NN):
    return jax.lax.dot_general(a, b, dims, preferred_element_type=_F32)


def _layernorm(x, eps=1e-05):
    m = jnp.mean(x, axis=-1, keepdims=True)
    xc = x - m
    v = jnp.mean(xc * xc, axis=-1, keepdims=True)
    return xc / jnp.sqrt(v + eps)


def _kernel(
    x_hbm, c_hbm, wmod_hbm, wq_hbm, wuk_hbm, ckv_hbm, wuv_hbm, wo_hbm,
    wg_hbm, wu_hbm, wd_hbm,
    o_ref,
    x_v, c_v, wmod_v, wq_v, wuk_v, ckv_v, wuv_v, wo_v, wg_v, wu_v, wd_v,
    e_v, sems, kv_sems,
    *, n_heads, d_head,
):
    H, D = n_heads, d_head
    Sk, Dc = ckv_v.shape
    M = x_v.shape[-1]
    Df = wd_v.shape[0]
    n_kv = Sk // _KV_CHUNK
    grp = _LANES * H

    def kv_copy(i):
        rows = pl.ds(pl.multiple_of(i * _KV_CHUNK, _KV_CHUNK), _KV_CHUNK)
        return pltpu.make_async_copy(ckv_hbm.at[rows], ckv_v.at[rows], kv_sems.at[i])

    def copy(src, dst, k):
        return pltpu.make_async_copy(src, dst, sems.at[k])

    d0 = Df - _DOWN_TAIL
    cp_x = copy(x_hbm, x_v, 0)
    cp_c = copy(c_hbm, c_v, 1)
    cp_mod = copy(wmod_hbm, wmod_v, 2)
    cp_q = copy(wq_hbm, wq_v, 3)
    cp_uk = copy(wuk_hbm, wuk_v, 4)
    cp_uv = copy(wuv_hbm, wuv_v, 5)
    cp_o = copy(wo_hbm, wo_v, 6)
    cp_g = copy(wg_hbm, wg_v, 7)
    cp_u = copy(wu_hbm, wu_v, 8)
    cp_d0 = copy(wd_hbm.at[pl.ds(0, d0)], wd_v.at[pl.ds(0, d0)], 9)
    cp_d1 = copy(wd_hbm.at[pl.ds(d0, _DOWN_TAIL)], wd_v.at[pl.ds(d0, _DOWN_TAIL)], 10)

    for cp in (cp_mod, cp_c, cp_x, cp_q, cp_uk):
        cp.start()
    for i in range(n_kv):
        kv_copy(i).start()
    for cp in (cp_uv, cp_o, cp_g, cp_u, cp_d0, cp_d1):
        cp.start()

    e_row = jax.lax.broadcasted_iota(jnp.int32, (_LANES, grp), 0)
    e_col = jax.lax.broadcasted_iota(jnp.int32, (_LANES, grp), 1)
    e_v[...] = jnp.where(e_col // H == e_row, 1.0, 0.0).astype(_BF16)
    hh = jax.lax.broadcasted_iota(jnp.int32, (H, grp), 0)
    jj = jax.lax.broadcasted_iota(jnp.int32, (H, grp), 1)
    diag = (jj % H) == hh

    def per_head_contract_rows(a, w_v):
        n_t = a.shape[1] // _LANES
        out = jnp.zeros((H, D), _F32)
        for t in range(n_t):
            rep = _dot(a[:, t * _LANES:(t + 1) * _LANES], e_v[...])
            lhs = jnp.where(diag, rep, 0.0).astype(_BF16)
            out = out + _dot(lhs, w_v[t * grp:(t + 1) * grp, :])
        return out

    cp_c.wait()
    cp_x.wait()
    cp_mod.wait()
    c = c_v[...].astype(_F32)
    silu_c = (c * jax.nn.sigmoid(c)).astype(_BF16)
    mod = _dot(silu_c, wmod_v[...])
    sa, ca, ga, sb, cb, gb = [mod[:, i * M:(i + 1) * M] for i in range(6)]
    x = x_v[...].astype(_F32)
    h1 = (_layernorm(x) * (1.0 + ca) + sa).astype(_BF16)

    cp_q.wait()
    q = per_head_contract_rows(jnp.broadcast_to(h1, (H, M)), wq_v).astype(_BF16)

    cp_uk.wait()
    scale = D ** (-0.5)
    parts = []
    for t in range(Dc // _LANES):
        r = _dot(q, wuk_v[t * grp:(t + 1) * grp, :], _NT)
        r = jnp.where(diag, r * scale, 0.0).astype(_BF16)
        parts.append(_dot(r, e_v[...], _NT))
    qa = jnp.concatenate(parts, axis=1).astype(_BF16)

    def kv_step(i, carry):
        kv_copy(i).wait()
        for j in range(_KV_CHUNK // _KV_TILE):
            m, l, acc = carry
            start = pl.multiple_of(i * _KV_CHUNK + j * _KV_TILE, _KV_TILE)
            kv = ckv_v[pl.ds(start, _KV_TILE), :]
            s = _dot(qa, kv, _NT)
            m_new = jnp.maximum(m, jnp.max(s, axis=1, keepdims=True))
            alpha = jnp.exp(m - m_new)
            p = jnp.exp(s - m_new)
            l = alpha * l + jnp.sum(p, axis=1, keepdims=True)
            acc = alpha * acc + _dot(p.astype(_BF16), kv)
            carry = (m_new, l, acc)
        return carry

    init = (
        jnp.full((H, 1), -jnp.inf, _F32),
        jnp.zeros((H, 1), _F32),
        jnp.zeros((H, Dc), _F32),
    )
    _, l, acc = jax.lax.fori_loop(0, n_kv, kv_step, init)
    lat = (acc / l).astype(_BF16)

    cp_uv.wait()
    ctx = per_head_contract_rows(lat, wuv_v)
    blk = (
        jax.lax.broadcasted_iota(jnp.int32, (H, H * D), 1) // D
        == jax.lax.broadcasted_iota(jnp.int32, (H, H * D), 0)
    )
    ctx_bd = jnp.where(blk, jnp.concatenate([ctx] * H, axis=1), 0.0).astype(_BF16)
    cp_o.wait()
    attn = jnp.sum(_dot(ctx_bd, wo_v[...]), axis=0, keepdims=True)
    x = x + ga * attn

    h2 = (_layernorm(x) * (1.0 + cb) + sb).astype(_BF16)
    cp_g.wait()
    g = jax.nn.gelu(_dot(h2, wg_v[...]), approximate=True)
    cp_u.wait()
    hid = (g * _dot(h2, wu_v[...])).astype(_BF16)
    cp_d0.wait()
    y = _dot(hid[:, :d0], wd_v[0:d0, :])
    cp_d1.wait()
    y = y + _dot(hid[:, d0:], wd_v[d0:Df, :])
    o_ref[...] = (x + gb * y).astype(o_ref.dtype)


@jax.jit
def pallas_adaLN_cond__compressed_kv_cla__glu_gated_geglu__decode_kernel(
    A_x: jax.Array,
    A_c_kv: jax.Array,
    A_w_q: jax.Array,
    A_w_uk: jax.Array,
    A_w_uv: jax.Array,
    A_w_o: jax.Array,
    B_x: jax.Array,
    B_w_gate: jax.Array,
    B_w_up: jax.Array,
    B_w_down: jax.Array,
    c: jax.Array,
    w_mod: jax.Array,
):
    B, Sq, M = A_x.shape
    assert B == 1 and Sq == 1
    Sk, Dc = A_c_kv.shape[1], A_c_kv.shape[2]
    H, D = A_w_q.shape[1], A_w_q.shape[2]

    operands = (
        A_x.reshape(1, M),
        c,
        w_mod,
        A_w_q.reshape(M * H, D),
        A_w_uk.reshape(Dc * H, D),
        A_c_kv.reshape(Sk, Dc),
        A_w_uv.reshape(Dc * H, D),
        A_w_o.reshape(H * D, M),
        B_w_gate,
        B_w_up,
        B_w_down,
    )
    scratch = [pltpu.VMEM(a.shape, a.dtype) for a in operands]
    scratch += [
        pltpu.VMEM((_LANES, _LANES * H), _BF16),
        pltpu.SemaphoreType.DMA((11,)),
        pltpu.SemaphoreType.DMA((Sk // _KV_CHUNK,)),
    ]
    out = pl.pallas_call(
        functools.partial(_kernel, n_heads=H, d_head=D),
        in_specs=[pl.BlockSpec(memory_space=pl.ANY)] * len(operands),
        out_specs=pl.BlockSpec(memory_space=pltpu.VMEM),
        out_shape=jax.ShapeDtypeStruct((1, M), A_x.dtype),
        scratch_shapes=scratch,
        compiler_params=pltpu.CompilerParams(vmem_limit_bytes=100 * 1024 * 1024),
    )(*operands)
    return out.reshape(B, Sq, M)
```

```python
import functools

import jax
import jax.numpy as jnp
import jax.experimental.pallas as pl
import jax.experimental.pallas.tpu as pltpu

_F32 = jnp.float32
_BF16 = jnp.bfloat16
_NN = (((1,), (0,)), ((), ()))
_NT = (((1,), (1,)), ((), ()))

_KV_CHUNK = 4096
_KV_TILE = 2048
_DOWN_TAIL = 256
_LANES = 128
_N_FIXED = 11


def _dot(a, b, dims=_NN):
    return jax.lax.dot_general(a, b, dims, preferred_element_type=_F32)


def _layernorm(x, eps=1e-05):
    m = jnp.mean(x, axis=-1, keepdims=True)
    xc = x - m
    v = jnp.mean(xc * xc, axis=-1, keepdims=True)
    return xc / jnp.sqrt(v + eps)


def _kernel(
    x_hbm, c_hbm, wmod_hbm, wq_hbm, wuk_hbm, ckv_hbm, wuv_hbm, wo_hbm,
    wg_hbm, wu_hbm, wd_hbm,
    o_ref,
    x_v, c_v, wmod_v, wq_v, wuk_v, ckv_v, wuv_v, wo_v, wg_v, wu_v, wd_v,
    e_v, sems,
    *, n_heads, d_head,
):
    H, D = n_heads, d_head
    Sk, Dc = ckv_v.shape
    M = x_v.shape[-1]
    Df = wd_v.shape[0]
    n_kv = Sk // _KV_CHUNK
    grp = _LANES * H

    def kv_copy(i):
        rows = pl.ds(pl.multiple_of(i * _KV_CHUNK, _KV_CHUNK), _KV_CHUNK)
        return pltpu.make_async_copy(ckv_hbm.at[rows], ckv_v.at[rows], sems.at[_N_FIXED + i])

    def copy(src, dst, k):
        return pltpu.make_async_copy(src, dst, sems.at[k])

    d0 = Df - _DOWN_TAIL
    cp_x = copy(x_hbm, x_v, 0)
    cp_c = copy(c_hbm, c_v, 1)
    cp_mod = copy(wmod_hbm, wmod_v, 2)
    cp_q = copy(wq_hbm, wq_v, 3)
    cp_uk = copy(wuk_hbm, wuk_v, 4)
    cp_uv = copy(wuv_hbm, wuv_v, 5)
    cp_o = copy(wo_hbm, wo_v, 6)
    cp_g = copy(wg_hbm, wg_v, 7)
    cp_u = copy(wu_hbm, wu_v, 8)
    cp_d0 = copy(wd_hbm.at[pl.ds(0, d0)], wd_v.at[pl.ds(0, d0)], 9)
    cp_d1 = copy(wd_hbm.at[pl.ds(d0, _DOWN_TAIL)], wd_v.at[pl.ds(d0, _DOWN_TAIL)], 10)

    for cp in (cp_mod, cp_c, cp_x, cp_q, cp_uk):
        cp.start()
    for i in range(n_kv):
        kv_copy(i).start()
    for cp in (cp_uv, cp_o, cp_g, cp_u, cp_d0, cp_d1):
        cp.start()

    e_row = jax.lax.broadcasted_iota(jnp.int32, (_LANES, grp), 0)
    e_col = jax.lax.broadcasted_iota(jnp.int32, (_LANES, grp), 1)
    e_v[...] = jnp.where(e_col // H == e_row, 1.0, 0.0).astype(_BF16)
    hh = jax.lax.broadcasted_iota(jnp.int32, (H, grp), 0)
    jj = jax.lax.broadcasted_iota(jnp.int32, (H, grp), 1)
    diag = (jj % H) == hh

    def per_head_contract_rows(a, w_v):
        n_t = a.shape[1] // _LANES
        out = jnp.zeros((H, D), _F32)
        for t in range(n_t):
            rep = _dot(a[:, t * _LANES:(t + 1) * _LANES], e_v[...])
            lhs = jnp.where(diag, rep, 0.0).astype(_BF16)
            out = out + _dot(lhs, w_v[t * grp:(t + 1) * grp, :])
        return out

    cp_c.wait()
    cp_x.wait()
    cp_mod.wait()
    c = c_v[...].astype(_F32)
    silu_c = (c * jax.nn.sigmoid(c)).astype(_BF16)
    mod = _dot(silu_c, wmod_v[...])
    sa, ca, ga, sb, cb, gb = [mod[:, i * M:(i + 1) * M] for i in range(6)]
    x = x_v[...].astype(_F32)
    h1 = (_layernorm(x) * (1.0 + ca) + sa).astype(_BF16)

    cp_q.wait()
    q = per_head_contract_rows(jnp.broadcast_to(h1, (H, M)), wq_v).astype(_BF16)

    cp_uk.wait()
    scale = D ** (-0.5)
    parts = []
    for t in range(Dc // _LANES):
        r = _dot(q, wuk_v[t * grp:(t + 1) * grp, :], _NT)
        r = jnp.where(diag, r * scale, 0.0).astype(_BF16)
        parts.append(_dot(r, e_v[...], _NT))
    qa = jnp.concatenate(parts, axis=1).astype(_BF16)

    def kv_step(i, carry):
        kv_copy(i).wait()
        for j in range(_KV_CHUNK // _KV_TILE):
            m, l, acc = carry
            start = pl.multiple_of(i * _KV_CHUNK + j * _KV_TILE, _KV_TILE)
            kv = ckv_v[pl.ds(start, _KV_TILE), :]
            s = _dot(qa, kv, _NT)
            m_new = jnp.maximum(m, jnp.max(s, axis=1, keepdims=True))
            alpha = jnp.exp(m - m_new)
            p = jnp.exp(s - m_new)
            l = alpha * l + jnp.sum(p, axis=1, keepdims=True)
            acc = alpha * acc + _dot(p.astype(_BF16), kv)
            carry = (m_new, l, acc)
        return carry

    init = (
        jnp.full((H, 1), -jnp.inf, _F32),
        jnp.zeros((H, 1), _F32),
        jnp.zeros((H, Dc), _F32),
    )
    _, l, acc = jax.lax.fori_loop(0, n_kv, kv_step, init)
    lat = (acc / l).astype(_BF16)

    cp_uv.wait()
    ctx = per_head_contract_rows(lat, wuv_v)
    blk = (
        jax.lax.broadcasted_iota(jnp.int32, (H, H * D), 1) // D
        == jax.lax.broadcasted_iota(jnp.int32, (H, H * D), 0)
    )
    ctx_bd = jnp.where(blk, jnp.concatenate([ctx] * H, axis=1), 0.0).astype(_BF16)
    cp_o.wait()
    attn = jnp.sum(_dot(ctx_bd, wo_v[...]), axis=0, keepdims=True)
    x = x + ga * attn

    h2 = (_layernorm(x) * (1.0 + cb) + sb).astype(_BF16)
    cp_g.wait()
    g = jax.nn.gelu(_dot(h2, wg_v[...]), approximate=True)
    cp_u.wait()
    hid = (g * _dot(h2, wu_v[...])).astype(_BF16)
    cp_d0.wait()
    y = _dot(hid[:, :d0], wd_v[0:d0, :])
    cp_d1.wait()
    y = y + _dot(hid[:, d0:], wd_v[d0:Df, :])
    o_ref[...] = (x + gb * y).astype(o_ref.dtype)


@jax.jit
def pallas_adaLN_cond__compressed_kv_cla__glu_gated_geglu__decode_kernel(
    A_x: jax.Array,
    A_c_kv: jax.Array,
    A_w_q: jax.Array,
    A_w_uk: jax.Array,
    A_w_uv: jax.Array,
    A_w_o: jax.Array,
    B_x: jax.Array,
    B_w_gate: jax.Array,
    B_w_up: jax.Array,
    B_w_down: jax.Array,
    c: jax.Array,
    w_mod: jax.Array,
):
    B, Sq, M = A_x.shape
    assert B == 1 and Sq == 1
    Sk, Dc = A_c_kv.shape[1], A_c_kv.shape[2]
    H, D = A_w_q.shape[1], A_w_q.shape[2]

    operands = (
        A_x.reshape(1, M),
        c,
        w_mod,
        A_w_q.reshape(M * H, D),
        A_w_uk.reshape(Dc * H, D),
        A_c_kv.reshape(Sk, Dc),
        A_w_uv.reshape(Dc * H, D),
        A_w_o.reshape(H * D, M),
        B_w_gate,
        B_w_up,
        B_w_down,
    )
    scratch = [pltpu.VMEM(a.shape, a.dtype) for a in operands]
    scratch += [
        pltpu.VMEM((_LANES, _LANES * H), _BF16),
        pltpu.SemaphoreType.DMA((_N_FIXED + Sk // _KV_CHUNK,)),
    ]
    out = pl.pallas_call(
        functools.partial(_kernel, n_heads=H, d_head=D),
        in_specs=[pl.BlockSpec(memory_space=pl.ANY)] * len(operands),
        out_specs=pl.BlockSpec(memory_space=pltpu.VMEM),
        out_shape=jax.ShapeDtypeStruct((1, M), A_x.dtype),
        scratch_shapes=scratch,
        compiler_params=pltpu.CompilerParams(vmem_limit_bytes=100 * 1024 * 1024),
    )(*operands)
    return out.reshape(B, Sq, M)
```

```python
import functools

import jax
import jax.numpy as jnp
import jax.experimental.pallas as pl
import jax.experimental.pallas.tpu as pltpu

_F32 = jnp.float32
_BF16 = jnp.bfloat16
_NN = (((1,), (0,)), ((), ()))
_NT = (((1,), (1,)), ((), ()))
_LANES = 128

_Q1 = 25
_PREFILL = 4
_LOOK = 26
_TOP1, _TOP2, _CATCH = 7, 9, 4
_TILE_POS = 8
_TAIL_PRE, _TAIL_MID = 100, 40
_D_SPLIT = (128, 512, 128, 128)

_S_MOD, _S_Q, _S_UK, _S_UV, _S_O, _S_G, _S_U, _S_D0 = range(8)
_N_D = len(_D_SPLIT) + 1
_S_KV = _S_D0 + _N_D


def _dot(a, b, dims=_NN):
    return jax.lax.dot_general(a, b, dims, preferred_element_type=_F32)


def _layernorm(x, eps=1e-05):
    m = jnp.mean(x, axis=-1, keepdims=True)
    xc = x - m
    v = jnp.mean(xc * xc, axis=-1, keepdims=True)
    return xc / jnp.sqrt(v + eps)


def _body(
    x_hbm, c_hbm, wmod_hbm, wq_hbm, wuk_hbm, ckv_hbm, wuv_hbm, wo_hbm,
    wg_hbm, wu_hbm, wd_hbm,
    o_ref,
    x_v, c_v, wmod_v, wq_v, wuk_v, ckv_v, wuv_v, wo_v, wg_v, wu_v, wd_v, e_v,
    sems, H, D,
):
    n_pos, n_str, kv_r, Dc = ckv_v.shape
    M = x_v.shape[-1]
    dr = wd_v.shape[1]
    Df = 2 * dr
    grp = _LANES * H
    kv_tile = _TILE_POS * n_str * kv_r
    n_tiles = n_pos // _TILE_POS
    n_w = wq_v.shape[1] // 128

    def start(src, dst, s, prio):
        pltpu.make_async_copy(src, dst, sems.at[s]).start(priority=prio)

    def wait(buf, s):
        pltpu.make_async_copy(buf, buf, sems.at[s]).wait()

    def pair(src, dst, idx, s, p0=0):
        for sl, p in ((pl.ds(0, 1), p0), (pl.ds(1, 3), 1)):
            start(src.at[(sl,) + idx], dst.at[(sl,) + idx], s, p)

    def head_pos(p, p0=0):
        half = wmod_v.shape[2] // 2
        idx = (
            pl.ds(pl.multiple_of((p // 2) * 8, 8), 8),
            pl.ds(pl.multiple_of((p % 2) * half, 128), half),
        )
        pair(wmod_hbm, wmod_v, idx, _S_MOD, p0)
        rows = (pl.ds(pl.multiple_of(p * 128, 128), 128),)
        pair(wq_hbm, wq_v, rows, _S_Q, p0)
        pair(wuk_hbm, wuk_v, rows, _S_UK, p0)

    def kv_pos(p):
        rows = pl.ds(pl.multiple_of(p * kv_r, kv_r), kv_r)
        s = _S_KV + p // _TILE_POS
        for u0 in range(0, n_str, 4):
            for sl, pr in ((pl.ds(u0, 1), 0), (pl.ds(u0 + 1, 3), 1)):
                start(ckv_hbm.at[sl, rows], ckv_v.at[p, sl], s, pr)

    def uvo_pos(p):
        pair(wuv_hbm, wuv_v, (pl.ds(pl.multiple_of(p * 128, 128), 128),), _S_UV)
        pair(wo_hbm, wo_v, (pl.ds(pl.multiple_of(p * 32, 32), 32),), _S_O)

    def loop(lo, hi, fn):
        def body(p, carry):
            fn(p)
            return carry

        jax.lax.fori_loop(lo, hi, body, 0)

    def issue(lo, hi):
        if isinstance(lo, int) and isinstance(hi, int):
            if lo < n_pos:
                loop(lo, min(hi, n_pos), kv_pos)
            if hi > n_pos:
                loop(max(lo, n_pos) - n_pos, hi - n_pos, uvo_pos)
        else:
            loop(lo, jnp.minimum(hi, n_pos), kv_pos)
            loop(jnp.maximum(lo, n_pos) - n_pos, hi - n_pos, uvo_pos)

    gu = []
    for j in range(wg_v.shape[1] // 8):
        for s in range(2):
            for h, v, sem in ((wg_hbm, wg_v, _S_G), (wu_hbm, wu_v, _S_U)):
                idx = (s, pl.ds(j * 8, 8))
                gu.append((h.at[idx], v.at[idx], sem))

    def dpieces(r0, r1, streams, sem):
        return [
            (wd_hbm.at[s, pl.ds(r, 32)], wd_v.at[s, pl.ds(r, 32)], sem)
            for r in range(r0, r1, 32)
            for s in streams
        ]

    dch = []
    r = 0
    for k, n in enumerate(_D_SPLIT[:-1]):
        dch.append(dpieces(r, r + n, (0, 1), _S_D0 + k))
        r += n
    assert r + _D_SPLIT[-1] == dr
    dch.append(dpieces(r, dr, (0,), _S_D0 + _N_D - 2))
    dch.append(dpieces(r, dr, (1,), _S_D0 + _N_D - 1))
    order = []
    n0, k0 = len(dch[0]), 0
    for i, d in enumerate(gu):
        order.append(d)
        while k0 < n0 and (k0 + 1) * len(gu) <= (i + 1) * n0 + len(gu) // 2:
            order.append(dch[0][k0])
            k0 += 1
    assert k0 == n0
    for ch in dch[1:]:
        order += ch
    mid = order[_Q1:len(order) - _Q1]
    hi_p = order[:_Q1] + mid[1::2]
    lo_p = mid[0::2] + order[len(order) - _Q1:]
    tail = []
    for k in range(max(len(hi_p), len(lo_p))):
        if k < len(hi_p):
            tail.append(hi_p[k] + (0,))
        if k < len(lo_p):
            tail.append(lo_p[k] + (1,))

    def issue_tail(lo, hi):
        for d in tail[lo:hi]:
            start(*d)

    start(c_hbm, c_v, _S_MOD, 1)
    start(x_hbm, x_v, _S_MOD, 1)
    loop(0, _PREFILL, lambda p: head_pos(p, 1))
    loop(_PREFILL, n_w // 2, head_pos)
    e_row = jax.lax.broadcasted_iota(jnp.int32, (_LANES, grp), 0)
    e_col = jax.lax.broadcasted_iota(jnp.int32, (_LANES, grp), 1)
    e_v[...] = jnp.where(e_col // H == e_row, 1.0, 0.0).astype(_BF16)
    loop(n_w // 2, n_w, head_pos)
    issue(0, _LOOK)
    hh = jax.lax.broadcasted_iota(jnp.int32, (H, grp), 0)
    jj = jax.lax.broadcasted_iota(jnp.int32, (H, grp), 1)
    diag = (jj % H) == hh

    def per_head_contract_rows(a, w_v):
        out = jnp.zeros((H, D), _F32)
        for t in range(a.shape[1] // _LANES):
            rep = _dot(a[:, t * _LANES:(t + 1) * _LANES], e_v[...])
            lhs = jnp.where(diag, rep, 0.0).astype(_BF16)
            out = out + _dot(lhs, w_v[t])
        return out

    wait(c_v, _S_MOD)
    wait(x_v, _S_MOD)
    wait(wmod_v, _S_MOD)
    c = c_v[...].astype(_F32)
    silu_c = (c * jax.nn.sigmoid(c)).astype(_BF16)
    mod = _dot(silu_c, wmod_v[...].reshape(M, 6 * M))
    sa, ca, ga, sb, cb, gb = [mod[:, i * M:(i + 1) * M] for i in range(6)]
    x = x_v[...].astype(_F32)
    h1 = (_layernorm(x) * (1.0 + ca) + sa).astype(_BF16)

    wait(wq_v, _S_Q)
    q = per_head_contract_rows(jnp.broadcast_to(h1, (H, M)), wq_v).astype(_BF16)
    issue(_LOOK, _LOOK + _TOP1)
    wait(wuk_v, _S_UK)
    scale = D ** (-0.5)
    parts = []
    for t in range(Dc // _LANES):
        r = _dot(q, wuk_v[t], _NT)
        r = jnp.where(diag, r * scale, 0.0).astype(_BF16)
        parts.append(_dot(r, e_v[...], _NT))
    qa = jnp.concatenate(parts, axis=1).astype(_BF16)

    p0 = _LOOK + _TOP1 + _TOP2

    def ptr(i, mx=jnp.maximum):
        return mx(_TILE_POS * (i + 1) + _LOOK, p0 + _CATCH * i)

    def kv_step(i, carry):
        issue(jnp.where(i == 0, _LOOK + _TOP1, ptr(i - 1)), ptr(i))
        tile = ckv_v.at[pl.ds(pl.multiple_of(i * _TILE_POS, _TILE_POS), _TILE_POS)]
        wait(tile, _S_KV + i)
        m, l, acc = carry
        kv = tile[...].reshape(kv_tile, Dc)
        s = _dot(qa, kv, _NT)
        m_new = jnp.maximum(m, jnp.max(s, axis=1, keepdims=True))
        alpha = jnp.exp(m - m_new)
        p = jnp.exp(s - m_new)
        l = alpha * l + jnp.sum(p, axis=1, keepdims=True)
        acc = alpha * acc + _dot(p.astype(_BF16), kv)
        return m_new, l, acc

    init = (
        jnp.full((H, 1), -jnp.inf, _F32),
        jnp.zeros((H, 1), _F32),
        jnp.zeros((H, Dc), _F32),
    )
    _, l, acc = jax.lax.fori_loop(0, n_tiles, kv_step, init)
    lat = (acc / l).astype(_BF16)
    last = ptr(n_tiles - 1, max)
    assert last <= n_pos + n_w
    issue(last, n_pos + n_w)
    issue_tail(0, _TAIL_PRE)

    wait(wuv_v, _S_UV)
    ctx = per_head_contract_rows(lat, wuv_v)
    blk = (
        jax.lax.broadcasted_iota(jnp.int32, (H, H * D), 1) // D
        == jax.lax.broadcasted_iota(jnp.int32, (H, H * D), 0)
    )
    ctx_bd = jnp.where(blk, jnp.concatenate([ctx] * H, axis=1), 0.0).astype(_BF16)
    issue_tail(_TAIL_PRE, _TAIL_PRE + _TAIL_MID)
    wait(wo_v, _S_O)
    attn = jnp.sum(_dot(ctx_bd, wo_v[...].reshape(H * D, M)), axis=0, keepdims=True)
    x = x + ga * attn

    h2 = (_layernorm(x) * (1.0 + cb) + sb).astype(_BF16)
    issue_tail(_TAIL_PRE + _TAIL_MID, len(tail))
    wait(wg_v, _S_G)
    g = jax.nn.gelu(_dot(h2, wg_v[...].reshape(M, Df)), approximate=True)
    wait(wu_v, _S_U)
    hid = (g * _dot(h2, wu_v[...].reshape(M, Df))).astype(_BF16)
    n = _D_SPLIT[-1]
    tl = hid[:, Df - _LANES:].astype(_F32)
    rr = jax.lax.broadcasted_iota(jnp.int32, (n, _LANES), 0)
    cc = jax.lax.broadcasted_iota(jnp.int32, (n, _LANES), 1)
    col = jnp.sum(
        jnp.where(cc == rr + (_LANES - n), jnp.broadcast_to(tl, (n, _LANES)), 0.0),
        axis=1, keepdims=True,
    )
    colb = jnp.broadcast_to(col, (n, M)) * gb
    r = 0
    for k, n in enumerate(_D_SPLIT[:-1]):
        wait(wd_v.at[:, pl.ds(r, n)], _S_D0 + k)
        lhs = jnp.concatenate([hid[:, r:r + n], hid[:, dr + r:dr + r + n]], axis=1)
        x = x + gb * _dot(lhs, wd_v[:, r:r + n, :].reshape(2 * n, M))
        r += n
    n = _D_SPLIT[-1]
    wait(wd_v.at[0, pl.ds(r, n)], _S_D0 + _N_D - 2)
    x = x + gb * _dot(hid[:, r:r + n], wd_v[0, r:r + n, :])
    wait(wd_v.at[1, pl.ds(r, n)], _S_D0 + _N_D - 1)
    x = x + jnp.sum(colb * wd_v[1, r:r + n, :].astype(_F32), axis=0, keepdims=True)
    o_ref[...] = x.astype(o_ref.dtype)


def _kernel(*refs, H, D, n_sems):
    pl.run_scoped(
        lambda sems: _body(*refs, sems, H, D), pltpu.SemaphoreType.DMA((n_sems,))
    )


@jax.jit
def pallas_adaLN_cond__compressed_kv_cla__glu_gated_geglu__decode_kernel(
    A_x: jax.Array,
    A_c_kv: jax.Array,
    A_w_q: jax.Array,
    A_w_uk: jax.Array,
    A_w_uv: jax.Array,
    A_w_o: jax.Array,
    B_x: jax.Array,
    B_w_gate: jax.Array,
    B_w_up: jax.Array,
    B_w_down: jax.Array,
    c: jax.Array,
    w_mod: jax.Array,
):
    B, Sq, M = A_x.shape
    assert B == 1 and Sq == 1
    Sk, Dc = A_c_kv.shape[1], A_c_kv.shape[2]
    H, D = A_w_q.shape[1], A_w_q.shape[2]
    Df = B_w_down.shape[0]

    operands = (
        A_x.reshape(1, M),
        c,
        w_mod.reshape(4, M // 4, 6 * M),
        A_w_q.reshape(4, M * H // 4, D),
        A_w_uk.reshape(4, Dc * H // 4, D),
        A_c_kv.reshape(8, Sk // 8, Dc),
        A_w_uv.reshape(4, Dc * H // 4, D),
        A_w_o.reshape(4, H * D // 4, M),
        B_w_gate.reshape(2, M // 2, Df),
        B_w_up.reshape(2, M // 2, Df),
        B_w_down.reshape(2, Df // 2, M),
    )
    scratch = [pltpu.VMEM(a.shape, a.dtype) for a in operands]
    n_pos = Sk // (8 * 32)
    scratch[5] = pltpu.VMEM((n_pos, 8, 32, Dc), A_c_kv.dtype)
    scratch += [pltpu.VMEM((_LANES, _LANES * H), _BF16)]
    out = pl.pallas_call(
        functools.partial(_kernel, H=H, D=D, n_sems=_S_KV + n_pos // _TILE_POS),
        in_specs=[pl.BlockSpec(memory_space=pl.ANY)] * len(operands),
        out_specs=pl.BlockSpec(memory_space=pltpu.VMEM),
        out_shape=jax.ShapeDtypeStruct((1, M), A_x.dtype),
        scratch_shapes=scratch,
        compiler_params=pltpu.CompilerParams(
            vmem_limit_bytes=100 * 1024 * 1024, disable_bounds_checks=True
        ),
    )(*operands)
    return out.reshape(B, Sq, M)
```

```python
import functools

import jax
import jax.numpy as jnp
import jax.experimental.pallas as pl
import jax.experimental.pallas.tpu as pltpu

_F32 = jnp.float32
_BF16 = jnp.bfloat16
_NN = (((1,), (0,)), ((), ()))
_NT = (((1,), (1,)), ((), ()))
_LANES = 128

_BLK = 32768
_SHIFT_ROWS = 16
_OFF_FFN = 2048
_PREFILL = 25
_SKEW = 12
_PRE = (7, 3, 2, 3, 3, 2)
_POST = 3
_TAIL = (140, 40, 25)
_D_ROWS = (256, 1024, 256, 128, 128)

(_S_X, _S_MOD, _S_Q, _S_UKA, _S_UKB, _S_UV0, _S_UV, _S_O0, _S_OA, _S_OB,
 _S_G, _S_U, _S_D0) = range(13)
_S_KV = _S_D0 + len(_D_ROWS)


def _dot(a, b, dims=_NN):
    return jax.lax.dot_general(a, b, dims, preferred_element_type=_F32)


def _layernorm(x, eps=1e-05):
    m = jnp.mean(x, axis=-1, keepdims=True)
    xc = x - m
    v = jnp.mean(xc * xc, axis=-1, keepdims=True)
    return xc / jnp.sqrt(v + eps)


def _rects(shape, a, b):
    rows, cols = shape
    g_bytes = cols * 16
    out = []
    a, b = max(a, 0), min(b, rows * cols * 2)
    while a < b:
        g, o = divmod(a, g_bytes)
        if o == 0 and b - a >= g_bytes:
            n = (b - a) // g_bytes
            out.append((g * 8, n * 8, 0, cols))
            a += n * g_bytes
        else:
            e = min(b, (g + 1) * g_bytes)
            out.append((g * 8, 8, o // 16, (e - a) // 16))
            a = e
    if len(out) == 3 and out[0][2] == out[2][3]:
        (r0, _, c0, nc0), (r1, nr1, _, _), (_, _, _, nc2) = out
        out = [(r0, 8 + nr1, c0, nc0), (r1, nr1 + 8, 0, nc2)]
    return out


def _round_robin(lanes):
    keyed = []
    for k, lane in enumerate(lanes):
        for i, item in enumerate(lane):
            keyed.append(((i + (k + 0.5) / len(lanes)) / len(lane), k, item))
    keyed.sort(key=lambda t: t[:2])
    return [item for _, _, item in keyed]


def _ffn_blocks(src, dst, sem, lo, hi, lanes):
    blocks = []
    k = (lo + _OFF_FFN) // _BLK
    while k * _BLK - _OFF_FFN < hi:
        a, b = k * _BLK - _OFF_FFN, (k + 1) * _BLK - _OFF_FFN
        blocks.append(_rects(dst.shape, max(lo, a), min(hi, b)))
        k += 1
    if len(blocks) > 1 and sum(r[1] * r[3] for r in blocks[-1]) * 2 <= 4096:
        last = blocks.pop()
        blocks[-1] = blocks[-1] + last
    blocks = [(src, dst, rs, sem) for rs in blocks]
    per = -(-len(blocks) // lanes)
    return [blocks[i * per:(i + 1) * per] for i in range(lanes)]


def _body(
    x_hbm, c_hbm, wmod_hbm, wq_hbm, wuk_hbm, ckv_hbm, wuv_hbm, wo_hbm,
    wg_hbm, wu_hbm, wd_hbm,
    o_ref,
    x_v, c_v, wmod_v, wq_v, wuk_v, ckv_v, wuv_v, wo_v, wg_v, wu_v, wd_v,
    e_v, et_v, lhs_v,
    sems, H, D,
):
    Sk, Dc = ckv_v.shape
    M = x_v.shape[-1]
    Df = wd_v.shape[0]
    grp = _LANES * H
    kv_lane = Sk // 8
    o_lane = H * D // 4
    half = Dc // 2
    n_tiles = kv_lane // 128

    issued = [0, 0]

    def view(ref, rect):
        r0, nr, c0, nc = rect
        if not isinstance(r0, int):
            r0 = pl.multiple_of(r0, 8)
        return ref.at[pl.ds(r0, nr), pl.ds(c0, nc)]

    def start(src, dst, rect, s, prio):
        pltpu.make_async_copy(view(src, rect), view(dst, rect), sems.at[s]).start(
            priority=prio
        )

    def block(src, dst, rs, s):
        prio = 1
        if issued[0] >= _PREFILL:
            prio = issued[1]
            issued[1] ^= 1
        for r in rs:
            start(src, dst, r, s, prio)
        issued[0] += len(rs)

    def wait(buf, s, rs=None):
        for r in rs or [(0, buf.shape[0], 0, buf.shape[1])]:
            v = view(buf, r)
            pltpu.make_async_copy(v, v, sems.at[s]).wait()

    def blk128(r, n=1):
        if isinstance(r, int) and r == 0:
            return [(0, 128 * n - _SHIFT_ROWS, 0, D), (4 * grp - _SHIFT_ROWS, _SHIFT_ROWS, 0, D)]
        return [(r - _SHIFT_ROWS, 128 * n, 0, D)]

    def blk512(rows, r, n=1):
        if isinstance(r, int) and r == 0:
            return [(0, 32 * n - 8, half, half), (0, 32 * n, 0, half), (rows - 8, 8, half, half)]
        return [(r - 8, 32 * n, half, half), (r, 32 * n, 0, half)]

    def head_step(v):
        t = 2 * M
        mods = [
            [[(r, 8, 0, 2 * t)], [(r, 8, 2 * t, t), (r + 8, 8, 0, t)], [(r + 8, 8, t, 2 * t)]][k]
            for k in range(3)
            for r in (s * (M // 4) + v * 16 for s in range(4))
        ]
        for j in range(4):
            for s in range(4):
                rs = blk128(s * grp + (v * 4 + j) * 128)
                block(wq_hbm, wq_v, rs, _S_Q)
                block(wuk_hbm, wuk_v, rs, _S_UKA if s < 2 else _S_UKB)
                if j < 3:
                    block(wmod_hbm, wmod_v, mods[j * 4 + s], _S_MOD)

    def kv_pos(p):
        for u in range(8):
            block(ckv_hbm, ckv_v, blk512(Sk, u * kv_lane + p * 32), _S_KV + p // 4)

    def kv_wait(g):
        wait(ckv_v, _S_KV + g, [r for u in range(8) for r in blk512(Sk, u * kv_lane + g * 128, 4)])

    def uvo_pos(p):
        first = isinstance(p, int) and p == 0
        for s in range(4):
            sem = _S_O0 if first else (_S_OA if s < 2 else _S_OB)
            block(wo_hbm, wo_v, blk512(H * D, s * o_lane + p * 32), sem)
        for s in range(4):
            block(wuv_hbm, wuv_v, blk128(s * grp + p * 128), _S_UV0 if first else _S_UV)

    gate = _ffn_blocks(wg_hbm, wg_v, _S_G, 0, M * Df * 2, 4)
    up = _ffn_blocks(wu_hbm, wu_v, _S_U, 0, M * Df * 2, 4)
    gate_up = _round_robin([lane for pair in zip(gate, up) for lane in pair])
    down, r = [], 0
    for k, n in enumerate(_D_ROWS):
        lanes = 2 if n >= 256 else 1
        down.append(_round_robin(
            _ffn_blocks(wd_hbm, wd_v, _S_D0 + k, r * M * 2, (r + n) * M * 2, lanes)))
        r += n
    assert r == Df
    order = []
    for i, b in enumerate(gate_up):
        order.append(b)
        if down[0] and i % 3 == 2:
            order.append(down[0].pop(0))
    for chunk in down:
        order += chunk
    mid = order[_SKEW:len(order) - _SKEW]
    by_prio = (order[:_SKEW] + mid[1::2], mid[0::2] + order[len(order) - _SKEW:])
    tail = []
    for k in range(len(by_prio[1])):
        for prio, blocks in enumerate(by_prio):
            if k < len(blocks):
                src, dst, rs, sem = blocks[k]
                tail += [(src, dst, r, sem, prio) for r in rs]

    def issue_tail(n):
        for d in tail[:n]:
            start(*d)
        del tail[:n]

    kv_next = [0]

    def issue_kv(n):
        for p in range(kv_next[0], kv_next[0] + n):
            kv_pos(p)
        kv_next[0] += n

    cp_c = pltpu.make_async_copy(c_hbm, c_v, sems.at[_S_X])
    cp_x = pltpu.make_async_copy(x_hbm, x_v, sems.at[_S_X])
    cp_c.start(priority=1)
    cp_x.start(priority=1)
    issued[0] = 2
    head_step(0)
    iota = jax.lax.broadcasted_iota
    e_v[...] = jnp.where(
        iota(jnp.int32, (_LANES, grp), 1) // H == iota(jnp.int32, (_LANES, grp), 0), 1.0, 0.0
    ).astype(_BF16)
    et_v[...] = jnp.where(
        iota(jnp.int32, (grp, _LANES), 0) // H == iota(jnp.int32, (grp, _LANES), 1), 1.0, 0.0
    ).astype(_BF16)

    def head_loop(v, carry):
        head_step(v)
        return carry

    jax.lax.fori_loop(1, grp // 512, head_loop, 0)
    uvo_pos(0)
    issue_kv(_PRE[0])

    diag4 = iota(jnp.int32, (4 * H, grp), 1) % H == iota(jnp.int32, (4 * H, grp), 0) % H
    diag = diag4[:H]

    def expand(a):
        st = jnp.concatenate([a[:, t * _LANES:(t + 1) * _LANES] for t in range(4)], axis=0)
        lhs_v[...] = jnp.where(diag4, _dot(st, e_v[...]), 0.0).astype(_BF16)

    def contract(w_v):
        lhs = jnp.concatenate([lhs_v[t * H:(t + 1) * H, :] for t in range(4)], axis=1)
        return _dot(lhs, w_v[...])

    wait(wmod_v, _S_MOD)
    cp_c.wait()
    cp_x.wait()
    c = c_v[...].astype(_F32)
    silu_c = (c * jax.nn.sigmoid(c)).astype(_BF16)
    mod = _dot(silu_c, wmod_v[...])
    sa, ca, ga, sb, cb, gb = [mod[:, i * M:(i + 1) * M] for i in range(6)]
    x = x_v[...].astype(_F32)
    h1 = (_layernorm(x) * (1.0 + ca) + sa).astype(_BF16)

    wait(wq_v, _S_Q)
    issue_kv(_PRE[1])
    expand(jnp.broadcast_to(h1, (H, M)))
    wait(wuk_v, _S_UKA, blk128(0, 2 * H))
    issue_kv(_PRE[2])
    q = contract(wq_v).astype(_BF16)
    wait(wuk_v, _S_UKB, blk128(2 * grp, 2 * H))
    issue_kv(_PRE[3])
    scale = D ** (-0.5)

    def absorb(t):
        r = _dot(q, wuk_v[t * grp:(t + 1) * grp, :], _NT)
        lhs_v[t * H:(t + 1) * H, :] = jnp.where(diag, r * scale, 0.0).astype(_BF16)

    absorb(0)
    absorb(1)
    kv_wait(0)
    issue_kv(_PRE[4])
    absorb(2)
    absorb(3)
    wait(wo_v, _S_O0, [r for s in range(4) for r in blk512(H * D, s * o_lane)])
    issue_kv(_PRE[5])
    picked = _dot(lhs_v[...], et_v[...])
    qa = jnp.concatenate([picked[t * H:(t + 1) * H] for t in range(4)], axis=1).astype(_BF16)

    def kv_compute(i, carry):
        m, l, acc = carry
        base = pl.multiple_of(i * 128, 128)
        kv = jnp.concatenate(
            [ckv_v[pl.ds(u * kv_lane + base, 128), :] for u in range(8)], axis=0
        )
        s = _dot(qa, kv, _NT)
        m_new = jnp.maximum(m, jnp.max(s, axis=1, keepdims=True))
        alpha = jnp.exp(m - m_new)
        p = jnp.exp(s - m_new)
        l = alpha * l + jnp.sum(p, axis=1, keepdims=True)
        acc = alpha * acc + _dot(p.astype(_BF16), kv)
        return m_new, l, acc

    p0 = kv_next[0]
    assert p0 % 4 == 0 and p0 >= 8
    n_a = n_tiles - p0 // 4

    def loop_a(i, carry):
        kv_wait(i + 1)
        for k in range(4):
            kv_pos(p0 + 4 * i + k)
        return kv_compute(i, carry)

    def loop_b(i, carry):
        @pl.when(i < n_tiles - 1)
        def _():
            kv_wait(i + 1)

        for k in range(4):
            uvo_pos(1 + 4 * (i - n_a) + k)
        return kv_compute(i, carry)

    init = (
        jnp.full((H, 1), -jnp.inf, _F32),
        jnp.zeros((H, 1), _F32),
        jnp.zeros((H, Dc), _F32),
    )
    carry = jax.lax.fori_loop(0, n_a, loop_a, init)
    _, l, acc = jax.lax.fori_loop(n_a, n_tiles, loop_b, carry)
    pb = 1 + p0
    assert pb + _POST <= H
    for p in range(pb, pb + _POST):
        uvo_pos(p)
    expand((acc / l).astype(_BF16))
    wait(wuv_v, _S_UV0, [r for s in range(4) for r in blk128(s * grp)])
    for p in range(pb + _POST, H):
        uvo_pos(p)
    issue_tail(_TAIL[0])

    wait(wuv_v, _S_UV, [r for s in range(4) for r in blk128(s * grp + 128, H - 1)])
    ctx = contract(wuv_v)
    own = iota(jnp.int32, (H, H * D), 1) // D == iota(jnp.int32, (H, H * D), 0)
    ctx_bd = jnp.where(own, jnp.concatenate([ctx] * H, axis=1), 0.0).astype(_BF16)
    k2 = 2 * o_lane
    wait(wo_v, _S_OA, [r for s in (0, 1) for r in blk512(H * D, s * o_lane + 32, H - 1)])
    issue_tail(_TAIL[1])
    attn = jnp.sum(_dot(ctx_bd[:, :k2], wo_v[0:k2, :]), axis=0, keepdims=True)
    wait(wo_v, _S_OB, [r for s in (2, 3) for r in blk512(H * D, s * o_lane + 32, H - 1)])
    issue_tail(_TAIL[2])
    attn = attn + jnp.sum(_dot(ctx_bd[:, k2:], wo_v[k2:2 * k2, :]), axis=0, keepdims=True)
    x = x + ga * attn

    h2 = (_layernorm(x) * (1.0 + cb) + sb).astype(_BF16)
    assert all(d[3] != _S_D0 for d in tail)
    wait(wd_v, _S_D0, [(0, _D_ROWS[0], 0, M)])
    issue_tail(len(tail))
    wait(wg_v, _S_G)
    g = jax.nn.gelu(_dot(h2, wg_v[...]), approximate=True)
    wait(wu_v, _S_U)
    hid = (g * _dot(h2, wu_v[...])).astype(_BF16)
    n = _D_ROWS[-1]
    last = jnp.broadcast_to(hid[:, Df - _LANES:].astype(_F32), (n, _LANES))
    pick = iota(jnp.int32, (n, _LANES), 1) == iota(jnp.int32, (n, _LANES), 0) + (_LANES - n)
    col = jnp.sum(jnp.where(pick, last, 0.0), axis=1, keepdims=True)
    factor = jnp.broadcast_to(col, (n, M)) * gb
    r = 0
    for k, n in enumerate(_D_ROWS):
        if k > 0:
            wait(wd_v, _S_D0 + k, [(r, n, 0, M)])
        if k < len(_D_ROWS) - 1:
            x = x + gb * _dot(hid[:, r:r + n], wd_v[r:r + n, :])
        else:
            x = x + jnp.sum(factor * wd_v[r:r + n, :].astype(_F32), axis=0, keepdims=True)
        r += n
    o_ref[...] = x.astype(o_ref.dtype)


def _kernel(*refs, H, D, n_sems):
    pl.run_scoped(
        lambda sems: _body(*refs, sems, H, D), pltpu.SemaphoreType.DMA((n_sems,))
    )


@jax.jit
def pallas_adaLN_cond__compressed_kv_cla__glu_gated_geglu__decode_kernel(
    A_x: jax.Array,
    A_c_kv: jax.Array,
    A_w_q: jax.Array,
    A_w_uk: jax.Array,
    A_w_uv: jax.Array,
    A_w_o: jax.Array,
    B_x: jax.Array,
    B_w_gate: jax.Array,
    B_w_up: jax.Array,
    B_w_down: jax.Array,
    c: jax.Array,
    w_mod: jax.Array,
):
    B, Sq, M = A_x.shape
    Sk, Dc = A_c_kv.shape[1], A_c_kv.shape[2]
    H, D = A_w_q.shape[1], A_w_q.shape[2]
    assert (B, Sq, M, Dc, H, D) == (1, 1, 512, 512, 32, 128) and Sk % 1024 == 0

    operands = (
        A_x.reshape(1, M),
        c,
        w_mod,
        A_w_q.reshape(M * H, D),
        A_w_uk.reshape(Dc * H, D),
        A_c_kv.reshape(Sk, Dc),
        A_w_uv.reshape(Dc * H, D),
        A_w_o.reshape(H * D, M),
        B_w_gate,
        B_w_up,
        B_w_down,
    )
    scratch = [pltpu.VMEM(a.shape, a.dtype) for a in operands]
    scratch += [
        pltpu.VMEM((_LANES, _LANES * H), _BF16),
        pltpu.VMEM((_LANES * H, _LANES), _BF16),
        pltpu.VMEM((4 * H, _LANES * H), _BF16),
    ]
    out = pl.pallas_call(
        functools.partial(_kernel, H=H, D=D, n_sems=_S_KV + Sk // 1024),
        in_specs=[pl.BlockSpec(memory_space=pl.ANY)] * len(operands),
        out_specs=pl.BlockSpec(memory_space=pltpu.VMEM),
        out_shape=jax.ShapeDtypeStruct((1, M), A_x.dtype),
        scratch_shapes=scratch,
        compiler_params=pltpu.CompilerParams(
            vmem_limit_bytes=100 * 1024 * 1024, disable_bounds_checks=True
        ),
    )(*operands)
    return out.reshape(B, Sq, M)
```

```python
import functools

import jax
import jax.numpy as jnp
import jax.experimental.pallas as pl
import jax.experimental.pallas.tpu as pltpu

_F32 = jnp.float32
_BF16 = jnp.bfloat16
_NN = (((1,), (0,)), ((), ()))
_NT = (((1,), (1,)), ((), ()))
_LANES = 128

_BLK = 32768
_SHIFT_ROWS = 16
_OFF_FFN = 2048
_PREFILL = 27
_SKEW = 12
_PRE = (7, 3, 2, 3, 3, 2)
_POST = 3
_TAIL = (140, 40, 25)
_D_ROWS = (256, 1024, 256, 128, 96, 32)
_D_VPU = 3

(_S_X, _S_MOD, _S_Q, _S_UKA, _S_UKB, _S_UV0, _S_UV, _S_O0, _S_OA, _S_OB,
 _S_G, _S_U, _S_D0) = range(13)
_S_KV = _S_D0 + len(_D_ROWS)


def _dot(a, b, dims=_NN):
    return jax.lax.dot_general(a, b, dims, preferred_element_type=_F32)


def _layernorm(x, eps=1e-05):
    m = jnp.mean(x, axis=-1, keepdims=True)
    xc = x - m
    v = jnp.mean(xc * xc, axis=-1, keepdims=True)
    return xc / jnp.sqrt(v + eps)


def _rects(shape, a, b):
    rows, cols = shape
    g_bytes = cols * 16
    out = []
    a, b = max(a, 0), min(b, rows * cols * 2)
    while a < b:
        g, o = divmod(a, g_bytes)
        if o == 0 and b - a >= g_bytes:
            n = (b - a) // g_bytes
            out.append((g * 8, n * 8, 0, cols))
            a += n * g_bytes
        else:
            e = min(b, (g + 1) * g_bytes)
            out.append((g * 8, 8, o // 16, (e - a) // 16))
            a = e
    if len(out) == 3 and out[0][2] == out[2][3]:
        (r0, _, c0, nc0), (r1, nr1, _, _), (_, _, _, nc2) = out
        out = [(r0, 8 + nr1, c0, nc0), (r1, nr1 + 8, 0, nc2)]
    return out


def _round_robin(lanes):
    keyed = []
    for k, lane in enumerate(lanes):
        for i, item in enumerate(lane):
            keyed.append(((i + (k + 0.5) / len(lanes)) / len(lane), k, item))
    keyed.sort(key=lambda t: t[:2])
    return [item for _, _, item in keyed]


def _ffn_blocks(src, dst, sem, lo, hi, lanes, off=_OFF_FFN):
    blocks = []
    k = (lo + off) // _BLK
    while k * _BLK - off < hi:
        a, b = k * _BLK - off, (k + 1) * _BLK - off
        blocks.append(_rects(dst.shape, max(lo, a), min(hi, b)))
        k += 1
    if len(blocks) > 1 and sum(r[1] * r[3] for r in blocks[-1]) * 2 <= 4096:
        last = blocks.pop()
        blocks[-1] = blocks[-1] + last
    blocks = [(src, dst, rs, sem) for rs in blocks]
    per = -(-len(blocks) // lanes)
    return [blocks[i * per:(i + 1) * per] for i in range(lanes)]


def _body(
    x_hbm, c_hbm, wmod_hbm, wq_hbm, wuk_hbm, ckv_hbm, wuv_hbm, wo_hbm,
    wg_hbm, wu_hbm, wd_hbm,
    o_ref,
    x_v, c_v, wmod_v, wq_v, wuk_v, ckv_v, wuv_v, wo_v, wg_v, wu_v, wd_v,
    e_v, et_v, lhs_v,
    sems, H, D,
):
    Sk, Dc = ckv_v.shape
    M = x_v.shape[-1]
    Df = wd_v.shape[0]
    grp = _LANES * H
    kv_lane = Sk // 8
    o_lane = H * D // 4
    half = Dc // 2
    n_tiles = kv_lane // 128

    issued = [0, 0]

    def view(ref, rect):
        r0, nr, c0, nc = rect
        if not isinstance(r0, int):
            r0 = pl.multiple_of(r0, 8)
        return ref.at[pl.ds(r0, nr), pl.ds(c0, nc)]

    def start(src, dst, rect, s, prio):
        pltpu.make_async_copy(view(src, rect), view(dst, rect), sems.at[s]).start(
            priority=prio
        )

    def block(src, dst, rs, s):
        prio = 1
        if issued[0] >= _PREFILL:
            prio = issued[1]
            issued[1] ^= 1
        for r in rs:
            start(src, dst, r, s, prio)
        issued[0] += len(rs)

    def wait(buf, s, rs=None):
        for r in rs or [(0, buf.shape[0], 0, buf.shape[1])]:
            v = view(buf, r)
            pltpu.make_async_copy(v, v, sems.at[s]).wait()

    def blk128(r, n=1):
        if isinstance(r, int) and r == 0:
            return [(0, 128 * n - _SHIFT_ROWS, 0, D), (4 * grp - _SHIFT_ROWS, _SHIFT_ROWS, 0, D)]
        return [(r - _SHIFT_ROWS, 128 * n, 0, D)]

    def blk512(rows, r, n=1):
        if isinstance(r, int) and r == 0:
            return [(0, 32 * n - 8, half, half), (0, 32 * n, 0, half), (rows - 8, 8, half, half)]
        return [(r - 8, 32 * n, half, half), (r, 32 * n, 0, half)]

    def head_step(v):
        t = 2 * M
        mods = [
            [[(r, 8, 0, 2 * t)], [(r, 8, 2 * t, t), (r + 8, 8, 0, t)], [(r + 8, 8, t, 2 * t)]][k]
            for k in range(3)
            for r in (s * (M // 4) + v * 16 for s in range(4))
        ]
        for j in range(4):
            lanes = [blk128(s * grp + (v * 4 + j) * 128) for s in range(4)]
            for s, rs in enumerate(lanes):
                block(wuk_hbm, wuk_v, rs, _S_UKA if s < 2 else _S_UKB)
            for rs in lanes:
                block(wq_hbm, wq_v, rs, _S_Q)
            for rs in mods[j * 4:(j + 1) * 4]:
                block(wmod_hbm, wmod_v, rs, _S_MOD)

    def kv_row(u, r):
        if u % 2:
            r = (r + kv_lane // 2) % kv_lane
        return u * kv_lane + r

    def kv_pos(p):
        for u in range(8):
            block(ckv_hbm, ckv_v, blk512(Sk, kv_row(u, p * 32)), _S_KV + p // 4)

    def kv_wait(g):
        wait(ckv_v, _S_KV + g, [r for u in range(8) for r in blk512(Sk, kv_row(u, g * 128), 4)])

    def uvo_pos(p):
        first = isinstance(p, int) and p == 0
        for s in range(4):
            sem = _S_O0 if first else (_S_OA if s < 2 else _S_OB)
            block(wo_hbm, wo_v, blk512(H * D, s * o_lane + p * 32), sem)
        for s in range(4):
            block(wuv_hbm, wuv_v, blk128(s * grp + p * 128), _S_UV0 if first else _S_UV)

    gate = _ffn_blocks(wg_hbm, wg_v, _S_G, 0, M * Df * 2, 3)
    up = _ffn_blocks(wu_hbm, wu_v, _S_U, 0, M * Df * 2, 3)
    gate_up = _round_robin([lane for pair in zip(gate, up) for lane in pair])
    down, r = [], 0
    for k, n in enumerate(_D_ROWS):
        lanes = 2 if n >= 256 else 1
        off = _OFF_FFN if k < len(_D_ROWS) - 1 else 0
        down.append(_round_robin(
            _ffn_blocks(wd_hbm, wd_v, _S_D0 + k, r * M * 2, (r + n) * M * 2, lanes, off)))
        r += n
    assert r == Df
    order = []
    for i, b in enumerate(gate_up):
        order.append(b)
        if down[0] and i % 3 == 2:
            order.append(down[0].pop(0))
    for chunk in down:
        order += chunk
    mid = order[_SKEW:len(order) - _SKEW]
    by_prio = (order[:_SKEW] + mid[1::2], mid[0::2] + order[len(order) - _SKEW:])
    tail = []
    for k in range(len(by_prio[1])):
        for prio, blocks in enumerate(by_prio):
            if k < len(blocks):
                src, dst, rs, sem = blocks[k]
                tail += [(src, dst, r, sem, prio) for r in rs]

    def issue_tail(n):
        for d in tail[:n]:
            start(*d)
        del tail[:n]

    kv_next = [0]

    def issue_kv(n):
        for p in range(kv_next[0], kv_next[0] + n):
            kv_pos(p)
        kv_next[0] += n

    cp_c = pltpu.make_async_copy(c_hbm, c_v, sems.at[_S_X])
    cp_x = pltpu.make_async_copy(x_hbm, x_v, sems.at[_S_X])
    cp_c.start(priority=1)
    cp_x.start(priority=1)
    issued[0] = 2
    head_step(0)
    iota = jax.lax.broadcasted_iota
    e_v[...] = jnp.where(
        iota(jnp.int32, (_LANES, grp), 1) // H == iota(jnp.int32, (_LANES, grp), 0), 1.0, 0.0
    ).astype(_BF16)
    et_v[...] = jnp.where(
        iota(jnp.int32, (grp, _LANES), 0) // H == iota(jnp.int32, (grp, _LANES), 1), 1.0, 0.0
    ).astype(_BF16)

    def head_loop(v, carry):
        head_step(v)
        return carry

    jax.lax.fori_loop(1, grp // 512, head_loop, 0)
    uvo_pos(0)
    issue_kv(_PRE[0])

    diag4 = iota(jnp.int32, (4 * H, grp), 1) % H == iota(jnp.int32, (4 * H, grp), 0) % H
    diag = diag4[:H]

    def expand(a):
        st = jnp.concatenate([a[:, t * _LANES:(t + 1) * _LANES] for t in range(4)], axis=0)
        lhs_v[...] = jnp.where(diag4, _dot(st, e_v[...]), 0.0).astype(_BF16)

    def contract(w_v):
        lhs = jnp.concatenate([lhs_v[t * H:(t + 1) * H, :] for t in range(4)], axis=1)
        return _dot(lhs, w_v[...])

    wait(wmod_v, _S_MOD)
    cp_c.wait()
    cp_x.wait()
    c = c_v[...].astype(_F32)
    silu_c = (c * jax.nn.sigmoid(c)).astype(_BF16)
    mod = _dot(silu_c, wmod_v[...])
    sa, ca, ga, sb, cb, gb = [mod[:, i * M:(i + 1) * M] for i in range(6)]
    x = x_v[...].astype(_F32)
    h1 = (_layernorm(x) * (1.0 + ca) + sa).astype(_BF16)

    wait(wq_v, _S_Q)
    issue_kv(_PRE[1])
    expand(jnp.broadcast_to(h1, (H, M)))
    wait(wuk_v, _S_UKA, blk128(0, 2 * H))
    issue_kv(_PRE[2])
    q = contract(wq_v).astype(_BF16)
    wait(wuk_v, _S_UKB, blk128(2 * grp, 2 * H))
    issue_kv(_PRE[3])
    scale = D ** (-0.5)

    def absorb(t):
        r = _dot(q, wuk_v[t * grp:(t + 1) * grp, :], _NT)
        lhs_v[t * H:(t + 1) * H, :] = jnp.where(diag, r * scale, 0.0).astype(_BF16)

    absorb(0)
    absorb(1)
    kv_wait(0)
    issue_kv(_PRE[4])
    absorb(2)
    absorb(3)
    wait(wo_v, _S_O0, [r for s in range(4) for r in blk512(H * D, s * o_lane)])
    issue_kv(_PRE[5])
    picked = _dot(lhs_v[...], et_v[...])
    qa = jnp.concatenate([picked[t * H:(t + 1) * H] for t in range(4)], axis=1).astype(_BF16)

    def kv_compute(i, carry):
        m, l, acc = carry
        rows = [pl.multiple_of(kv_row(u, i * 128), 128) for u in range(8)]
        kv = jnp.concatenate([ckv_v[pl.ds(r, 128), :] for r in rows], axis=0)
        s = _dot(qa, kv, _NT)
        m_new = jnp.maximum(m, jnp.max(s, axis=1, keepdims=True))
        alpha = jnp.exp(m - m_new)
        p = jnp.exp(s - m_new)
        l = alpha * l + jnp.sum(p, axis=1, keepdims=True)
        acc = alpha * acc + _dot(p.astype(_BF16), kv)
        return m_new, l, acc

    p0 = kv_next[0]
    assert p0 % 4 == 0 and p0 >= 8
    n_a = n_tiles - p0 // 4

    def loop_a(i, carry):
        kv_wait(i + 1)
        for k in range(4):
            kv_pos(p0 + 4 * i + k)
        return kv_compute(i, carry)

    def loop_b(i, carry):
        @pl.when(i < n_tiles - 1)
        def _():
            kv_wait(i + 1)

        for k in range(4):
            uvo_pos(1 + 4 * (i - n_a) + k)
        return kv_compute(i, carry)

    init = (
        jnp.full((H, 1), -jnp.inf, _F32),
        jnp.zeros((H, 1), _F32),
        jnp.zeros((H, Dc), _F32),
    )
    carry = jax.lax.fori_loop(0, n_a, loop_a, init)
    _, l, acc = jax.lax.fori_loop(n_a, n_tiles, loop_b, carry)
    pb = 1 + p0
    assert pb + _POST <= H
    for p in range(pb, pb + _POST):
        uvo_pos(p)
    expand((acc / l).astype(_BF16))
    wait(wuv_v, _S_UV0, [r for s in range(4) for r in blk128(s * grp)])
    for p in range(pb + _POST, H):
        uvo_pos(p)
    issue_tail(_TAIL[0])

    wait(wuv_v, _S_UV, [r for s in range(4) for r in blk128(s * grp + 128, H - 1)])
    ctx = contract(wuv_v)
    own = iota(jnp.int32, (H, H * D), 1) // D == iota(jnp.int32, (H, H * D), 0)
    ctx_bd = jnp.where(own, jnp.concatenate([ctx] * H, axis=1), 0.0).astype(_BF16)
    k2 = 2 * o_lane
    wait(wo_v, _S_OA, [r for s in (0, 1) for r in blk512(H * D, s * o_lane + 32, H - 1)])
    issue_tail(_TAIL[1])
    attn = jnp.sum(_dot(ctx_bd[:, :k2], wo_v[0:k2, :]), axis=0, keepdims=True)
    wait(wo_v, _S_OB, [r for s in (2, 3) for r in blk512(H * D, s * o_lane + 32, H - 1)])
    issue_tail(_TAIL[2])
    attn = attn + jnp.sum(_dot(ctx_bd[:, k2:], wo_v[k2:2 * k2, :]), axis=0, keepdims=True)
    x = x + ga * attn

    h2 = (_layernorm(x) * (1.0 + cb) + sb).astype(_BF16)
    assert all(d[3] != _S_D0 for d in tail)
    wait(wd_v, _S_D0, [(0, _D_ROWS[0], 0, M)])
    issue_tail(len(tail))
    wait(wg_v, _S_G)
    g = jax.nn.gelu(_dot(h2, wg_v[...]), approximate=True)
    wait(wu_v, _S_U)
    hid = (g * _dot(h2, wu_v[...])).astype(_BF16)
    n_mxu = len(_D_ROWS) - _D_VPU
    nv = sum(_D_ROWS[n_mxu:])
    assert nv % _LANES == 0
    eye = iota(jnp.int32, (_LANES, _LANES), 0) == iota(jnp.int32, (_LANES, _LANES), 1)
    cols = []
    for r in range(Df - nv, Df, _LANES):
        part = jnp.broadcast_to(hid[:, r:r + _LANES].astype(_F32), (_LANES, _LANES))
        cols.append(jnp.sum(jnp.where(eye, part, 0.0), axis=1, keepdims=True))
    col = jnp.broadcast_to(jnp.concatenate(cols, axis=0), (nv, _LANES))
    col = jnp.concatenate([col] * (M // _LANES), axis=1)
    col_last = col[nv - _D_ROWS[-1]:] * gb
    y = jnp.zeros((8, M), _F32)
    r = 0
    for k, n in enumerate(_D_ROWS):
        last = k == len(_D_ROWS) - 1
        if last:
            first_row = iota(jnp.int32, (8, M), 0) == 0
            y = jnp.where(first_row, jnp.broadcast_to(x, (8, M)), 0.0) + gb * y
        if k > 0:
            wait(wd_v, _S_D0 + k, [(r, n, 0, M)])
        if k < n_mxu:
            x = x + gb * _dot(hid[:, r:r + n], wd_v[r:r + n, :])
        else:
            f = r - (Df - nv)
            prod = (col_last if last else col[f:f + n]) * wd_v[r:r + n, :].astype(_F32)
            for j in range(0, n, 8):
                y = y + prod[j:j + 8]
        r += n
    x = jnp.sum(y, axis=0, keepdims=True)
    o_ref[...] = x.astype(o_ref.dtype)


def _kernel(*refs, H, D, n_sems):
    pl.run_scoped(
        lambda sems: _body(*refs, sems, H, D), pltpu.SemaphoreType.DMA((n_sems,))
    )


@jax.jit
def pallas_adaLN_cond__compressed_kv_cla__glu_gated_geglu__decode_kernel(
    A_x: jax.Array,
    A_c_kv: jax.Array,
    A_w_q: jax.Array,
    A_w_uk: jax.Array,
    A_w_uv: jax.Array,
    A_w_o: jax.Array,
    B_x: jax.Array,
    B_w_gate: jax.Array,
    B_w_up: jax.Array,
    B_w_down: jax.Array,
    c: jax.Array,
    w_mod: jax.Array,
):
    B, Sq, M = A_x.shape
    Sk, Dc = A_c_kv.shape[1], A_c_kv.shape[2]
    H, D = A_w_q.shape[1], A_w_q.shape[2]
    assert (B, Sq, M, Dc, H, D) == (1, 1, 512, 512, 32, 128) and Sk % 2048 == 0

    operands = (
        A_x.reshape(1, M),
        c,
        w_mod,
        A_w_q.reshape(M * H, D),
        A_w_uk.reshape(Dc * H, D),
        A_c_kv.reshape(Sk, Dc),
        A_w_uv.reshape(Dc * H, D),
        A_w_o.reshape(H * D, M),
        B_w_gate,
        B_w_up,
        B_w_down,
    )
    scratch = [pltpu.VMEM(a.shape, a.dtype) for a in operands]
    scratch += [
        pltpu.VMEM((_LANES, _LANES * H), _BF16),
        pltpu.VMEM((_LANES * H, _LANES), _BF16),
        pltpu.VMEM((4 * H, _LANES * H), _BF16),
    ]
    out = pl.pallas_call(
        functools.partial(_kernel, H=H, D=D, n_sems=_S_KV + Sk // 1024),
        in_specs=[pl.BlockSpec(memory_space=pl.ANY)] * len(operands),
        out_specs=pl.BlockSpec(memory_space=pltpu.VMEM),
        out_shape=jax.ShapeDtypeStruct((1, M), A_x.dtype),
        scratch_shapes=scratch,
        compiler_params=pltpu.CompilerParams(
            vmem_limit_bytes=100 * 1024 * 1024, disable_bounds_checks=True
        ),
    )(*operands)
    return out.reshape(B, Sq, M)
```

```python
import functools

import jax
import jax.numpy as jnp
import jax.experimental.pallas as pl
import jax.experimental.pallas.tpu as pltpu

_F32 = jnp.float32
_BF16 = jnp.bfloat16
_NN = (((1,), (0,)), ((), ()))
_NT = (((1,), (1,)), ((), ()))
_LANES = 128

_BLK = 32768
_SHIFT_ROWS = 16
_OFF_FFN = 2048
_PREFILL = 27
_QUEUE = 25
_HEAD = "MUUQMQUUMQQ"
_PRE = (12, 6, 4, 6, 6, 6)
_POST = 6
_TAIL = (140, 40, 25)
_FFN_PHASES = (
    ({"g1": 8, "g2": 8, "g3": 8, "ug": 8, "d2": 2}, {"u1": 8, "u2": 8, "u3": 8, "d1": 3, "d3": 3}),
    ({"d2": 5, "d0": 3}, {"d1": 2, "d3": 3}),
    ({}, {"d1": 3, "d3": 2, "d2": 1, "d0": 1}),
)
_D_STAGES = (3, 15, 4, 3, 2, 1, 1)
_D_VPU = 4

(_S_X, _S_MOD, _S_Q, _S_UKA, _S_UKB, _S_UV0, _S_UV, _S_O0, _S_OA, _S_OB,
 _S_G, _S_U, _S_D0) = range(13)
_S_KV = _S_D0 + len(_D_STAGES)


def _dot(a, b, dims=_NN):
    return jax.lax.dot_general(a, b, dims, preferred_element_type=_F32)


def _layernorm(x, eps=1e-05):
    m = jnp.mean(x, axis=-1, keepdims=True)
    xc = x - m
    v = jnp.mean(xc * xc, axis=-1, keepdims=True)
    return xc / jnp.sqrt(v + eps)


def _rects(shape, a, b):
    rows, cols = shape
    g_bytes = cols * 16
    out = []
    a, b = max(a, 0), min(b, rows * cols * 2)
    while a < b:
        g, o = divmod(a, g_bytes)
        if o == 0 and b - a >= g_bytes:
            n = (b - a) // g_bytes
            out.append((g * 8, n * 8, 0, cols))
            a += n * g_bytes
        else:
            e = min(b, (g + 1) * g_bytes)
            out.append((g * 8, 8, o // 16, (e - a) // 16))
            a = e
    if len(out) == 3 and out[0][2] == out[2][3]:
        (r0, _, c0, nc0), (r1, nr1, _, _), (_, _, _, nc2) = out
        out = [(r0, 8 + nr1, c0, nc0), (r1, nr1 + 8, 0, nc2)]
    return out


def _round_robin(lanes):
    keyed = []
    for k, lane in enumerate(lanes):
        for i, item in enumerate(lane):
            keyed.append(((i + (k + 0.5) / len(lanes)) / len(lane), k, item))
    keyed.sort(key=lambda t: t[:2])
    return [item for _, _, item in keyed]


def _merge(ranges):
    out = []
    for lo, hi in ranges:
        if out and out[-1][1] == lo:
            out[-1] = (out[-1][0], hi)
        else:
            out.append((lo, hi))
    return out


def _ffn_plan(M, Df):
    shapes = {"g": (M, Df), "u": (M, Df), "d": (Df, M)}
    nb = M * Df * 2 // _BLK
    assert nb == 56

    def span(w, k):
        lo, hi = max(k * _BLK - _OFF_FFN, 0), (k + 1) * _BLK - _OFF_FFN
        if w == "d" and k < 2:
            lo, hi = (0, _BLK) if k == 0 else (_BLK, hi)
        return lo, (nb * _BLK if k == nb - 1 else hi)

    def units(w, k0, k1):
        return [[(w, k), (w, k + 1)] for k in range(k0, k1, 2)]

    regions = {
        "d0": units("d", 1, 9), "d1": units("d", 9, 25), "d2": units("d", 25, 41),
        "d3": [[("d", 55), ("u", 0)]] + units("d", 41, 55),
        "u1": units("u", 1, 17), "u2": units("u", 17, 33), "u3": units("u", 33, 49),
        "ug": [[("u", 55), ("g", 0)]] + units("g", 1, 9) + units("u", 49, 55),
        "g1": units("g", 9, 25), "g2": units("g", 25, 41),
        "g3": units("g", 41, 55) + [[("g", 55)]],
    }
    seqs = ([], [])
    for phase in _FFN_PHASES:
        for seq, counts in zip(seqs, phase):
            seq += _round_robin(
                [[regions[name].pop(0) for _ in range(n)] for name, n in counts.items()]
            )
    assert not any(regions.values())
    seqs[1].append([("d", 0)])
    blocks = [[blk for unit in seq for blk in unit] for seq in seqs]
    descs = [
        (blocks[prio][i], rect, prio)
        for i in range(max(map(len, blocks)))
        for prio in (0, 1)
        if i < len(blocks[prio])
        for rect in _rects(shapes[blocks[prio][i][0]], *span(*blocks[prio][i]))
    ]
    queue, arrival = [None] * _QUEUE, []
    for blk, _, prio in descs:
        if prio:
            queue.append(blk)
            blk = queue.pop(0)
        arrival.append(blk)
    when = {blk: i for i, blk in enumerate(arrival + queue)}
    down = sorted(
        (u for seq in seqs for u in seq if u[0][0] == "d"), key=lambda u: when[u[-1]]
    )
    assert sum(_D_STAGES) == len(down)
    stage = {}
    for k, n in enumerate(_D_STAGES):
        stage.update({b: k for u in down[:n] for w, b in u if w == "d"})
        del down[:n]
    sem = {"g": lambda b: _S_G, "u": lambda b: _S_U, "d": lambda b: _S_D0 + stage[b]}
    descs = [(w, rect, sem[w](b), prio) for (w, b), rect, prio in descs]
    fills, rows = [], [[] for _ in _D_STAGES]
    for k in range(len(_D_STAGES)):
        spans = _merge(span("d", b) for b in range(nb) if stage[b] == k)
        fills.append([r for lo, hi in spans for r in _rects(shapes["d"], lo, hi)])
    for r in range(0, Df, 16):
        lo, hi = r * M * 2, (r + 16) * M * 2
        need = [stage[b] for b in range(nb) if span("d", b)[0] < hi and span("d", b)[1] > lo]
        rows[max(need + [1])].append((r, r + 16))
    return descs, fills, [_merge(r) for r in rows]


def _body(
    x_hbm, c_hbm, wmod_hbm, wq_hbm, wuk_hbm, ckv_hbm, wuv_hbm, wo_hbm,
    wg_hbm, wu_hbm, wd_hbm,
    o_ref,
    x_v, c_v, wmod_v, wq_v, wuk_v, ckv_v, wuv_v, wo_v, wg_v, wu_v, wd_v,
    e_v, et_v, lhs_v,
    sems, H, D,
):
    Sk, Dc = ckv_v.shape
    M = x_v.shape[-1]
    Df = wd_v.shape[0]
    grp = _LANES * H
    half = Dc // 2
    n_tiles = Sk // 1024
    kv_lane = 4 * n_tiles
    w_lane = 32

    issued = [0]

    def view(ref, rect, shift=0):
        r0, nr, c0, nc = rect
        if isinstance(r0, int):
            r0 = (r0 + shift) % ref.shape[0]
        else:
            r0 = pl.multiple_of(r0 + shift, 8)
        return ref.at[pl.ds(r0, nr), pl.ds(c0, nc)]

    def start(src, dst, rect, s, prio, shift=0):
        pltpu.make_async_copy(view(src, rect, shift), view(dst, rect), sems.at[s]).start(
            priority=prio
        )

    def pair(src, dst, unit_a, unit_b, s, shift=0):
        order = [(unit_a[0], 0), (unit_b[0], 1), (unit_a[1], 0), (unit_b[1], 1)]
        if issued[0] < _PREFILL:
            order = [(rs, 1) for rs in unit_a + unit_b]
        for rs, prio in order:
            for r in rs:
                start(src, dst, r, s, prio, shift)
            issued[0] += len(rs)

    def wait(buf, s, rs=None):
        for r in rs or [(0, buf.shape[0], 0, buf.shape[1])]:
            v = view(buf, r)
            pltpu.make_async_copy(v, v, sems.at[s]).wait()

    def cut(rect, at):
        r0, nr, c0, nc = rect
        if not isinstance(r0, int):
            return [rect]
        rows = [r0] + [r for r in at if r0 < r < r0 + nr] + [r0 + nr]
        return [(a, b - a, c0, nc) for a, b in zip(rows, rows[1:])]

    def blk128(k, n=1):
        return cut((k * 128 - _SHIFT_ROWS, 128 * n, 0, D), (0,))

    def blk512(k, n=1, at=(0,)):
        return cut((k * 32 - 8, 32 * n, half, half), at) + cut((k * 32, 32 * n, 0, half), at)

    def w_pair(src, dst, blk, j, w, s):
        a, b = [[blk(u * w_lane + 2 * j + k) for k in (-1, 0)] for u in (2 * w, 2 * w + 1)]
        pair(src, dst, a, b, s)

    def mod_unit(r, j):
        t = 2 * M
        return [
            [[(r - 8, 8, t, 2 * t)], [(r, 8, 0, 2 * t)]],
            [[(r, 8, 2 * t, t), (r + 8, 8, 0, t)], [(r + 8, 8, t, 2 * t)]],
            [[(r + 16, 8, 0, 2 * t)], [(r + 16, 8, 2 * t, t), (r + 24, 8, 0, t)]],
        ][j]

    def head_step(v):
        for i, name in enumerate(_HEAD):
            n = _HEAD[:i].count(name)
            if name == "M":
                r = (v + 3 * n) % 8 * 32
                pair(wmod_hbm, wmod_v, mod_unit(r, n), mod_unit(M // 2 + r, n), _S_MOD)
            elif name == "U":
                w_pair(wuk_hbm, wuk_v, blk128, 2 * v + n // 2, n % 2, _S_UKA + n % 2)
            else:
                w_pair(wq_hbm, wq_v, blk128, 2 * v + n // 2, n % 2, _S_Q)

    def kv_pair(g, i):
        a, b = [
            [blk512(u * kv_lane + 4 * g + i // 4 * 2 + k, 1, (0, 32)) for k in (0, 1)]
            for u in (i % 4 * 2, i % 4 * 2 + 1)
        ]
        pair(ckv_hbm, ckv_v, a, b, _S_KV + g, -32)

    def kv_wait(g):
        wait(ckv_v, _S_KV + g, [r for u in range(8) for r in blk512(u * kv_lane + 4 * g, 4)])

    def uvo_pair(j, i):
        first = isinstance(j, int) and j == 0
        if i < 2:
            w_pair(wo_hbm, wo_v, blk512, j, i, _S_O0 if first else _S_OA + i)
        else:
            w_pair(wuv_hbm, wuv_v, blk128, j, i - 2, _S_UV0 if first else _S_UV)

    tail, d_fills, d_rows = _ffn_plan(M, Df)
    ffn = {"g": (wg_hbm, wg_v), "u": (wu_hbm, wu_v), "d": (wd_hbm, wd_v)}

    def issue_tail(n):
        for w, rect, s, prio in tail[:n]:
            start(*ffn[w], rect, s, prio)
        del tail[:n]

    kv_next = [0]

    def issue_kv(n):
        for i in range(kv_next[0], kv_next[0] + n):
            kv_pair(i // 8, i % 8)
        kv_next[0] += n

    cp_c = pltpu.make_async_copy(c_hbm, c_v, sems.at[_S_X])
    cp_x = pltpu.make_async_copy(x_hbm, x_v, sems.at[_S_X])
    cp_c.start(priority=1)
    cp_x.start(priority=1)
    issued[0] = 2
    head_step(0)
    iota = jax.lax.broadcasted_iota
    e_v[...] = jnp.where(
        iota(jnp.int32, (_LANES, grp), 1) // H == iota(jnp.int32, (_LANES, grp), 0), 1.0, 0.0
    ).astype(_BF16)
    et_v[...] = jnp.where(
        iota(jnp.int32, (grp, _LANES), 0) // H == iota(jnp.int32, (grp, _LANES), 1), 1.0, 0.0
    ).astype(_BF16)

    def head_loop(v, carry):
        head_step(v)
        return carry

    jax.lax.fori_loop(1, w_lane // 4, head_loop, 0)
    for i in range(4):
        uvo_pair(0, i)
    issue_kv(_PRE[0])

    diag4 = iota(jnp.int32, (4 * H, grp), 1) % H == iota(jnp.int32, (4 * H, grp), 0) % H
    diag = diag4[:H]

    def expand(a):
        st = jnp.concatenate([a[:, t * _LANES:(t + 1) * _LANES] for t in range(4)], axis=0)
        lhs_v[...] = jnp.where(diag4, _dot(st, e_v[...]), 0.0).astype(_BF16)

    def contract(w_v):
        lhs = jnp.concatenate([lhs_v[t * H:(t + 1) * H, :] for t in range(4)], axis=1)
        return _dot(lhs, w_v[...])

    wait(wmod_v, _S_MOD)
    cp_c.wait()
    cp_x.wait()
    c = c_v[...].astype(_F32)
    silu_c = (c * jax.nn.sigmoid(c)).astype(_BF16)
    mod = _dot(silu_c, wmod_v[...])
    sa, ca, ga, sb, cb, gb = [mod[:, i * M:(i + 1) * M] for i in range(6)]
    x = x_v[...].astype(_F32)
    h1 = (_layernorm(x) * (1.0 + ca) + sa).astype(_BF16)

    wait(wq_v, _S_Q)
    issue_kv(_PRE[1])
    expand(jnp.broadcast_to(h1, (H, M)))
    wait(wuk_v, _S_UKA, blk128(-1, 2 * w_lane))
    issue_kv(_PRE[2])
    q = contract(wq_v).astype(_BF16)
    wait(wuk_v, _S_UKB, blk128(2 * w_lane - 1, 2 * w_lane))
    issue_kv(_PRE[3])
    scale = D ** (-0.5)

    def absorb(t):
        r = _dot(q, wuk_v[t * grp:(t + 1) * grp, :], _NT)
        lhs_v[t * H:(t + 1) * H, :] = jnp.where(diag, r * scale, 0.0).astype(_BF16)

    absorb(0)
    absorb(1)
    assert kv_next[0] >= 8
    kv_wait(0)
    issue_kv(_PRE[4])
    absorb(2)
    absorb(3)
    wait(wo_v, _S_O0, [r for u in range(4) for r in blk512(u * w_lane - 1, 2)])
    issue_kv(_PRE[5])
    picked = _dot(lhs_v[...], et_v[...])
    qa = jnp.concatenate([picked[t * H:(t + 1) * H] for t in range(4)], axis=1).astype(_BF16)

    def kv_compute(i, carry):
        m, l, acc = carry
        rows = [pl.multiple_of(u * (Sk // 8) + i * 128, 128) for u in range(8)]
        kv = jnp.concatenate([ckv_v[pl.ds(r, 128), :] for r in rows], axis=0)
        s = _dot(qa, kv, _NT)
        m_new = jnp.maximum(m, jnp.max(s, axis=1, keepdims=True))
        alpha = jnp.exp(m - m_new)
        p = jnp.exp(s - m_new)
        l = alpha * l + jnp.sum(p, axis=1, keepdims=True)
        acc = alpha * acc + _dot(p.astype(_BF16), kv)
        return m_new, l, acc

    assert kv_next[0] % 8 == 0 and kv_next[0] >= 16
    g0 = kv_next[0] // 8
    n_a = n_tiles - g0

    def loop_a(i, carry):
        kv_wait(i + 1)
        for k in range(8):
            kv_pair(g0 + i, k)
        return kv_compute(i, carry)

    def loop_b(i, carry):
        @pl.when(i < n_tiles - 1)
        def _():
            kv_wait(i + 1)

        for k in range(8):
            uvo_pair(1 + 2 * (i - n_a) + k // 4, k % 4)
        return kv_compute(i, carry)

    init = (
        jnp.full((H, 1), -jnp.inf, _F32),
        jnp.zeros((H, 1), _F32),
        jnp.zeros((H, Dc), _F32),
    )
    carry = jax.lax.fori_loop(0, n_a, loop_a, init)
    _, l, acc = jax.lax.fori_loop(n_a, n_tiles, loop_b, carry)
    rest = list(range(4 + 8 * g0, 2 * w_lane))
    for i in rest[:_POST]:
        uvo_pair(i // 4, i % 4)
    expand((acc / l).astype(_BF16))
    wait(wuv_v, _S_UV0, [r for u in range(4) for r in blk128(u * w_lane - 1, 2)])
    for i in rest[_POST:]:
        uvo_pair(i // 4, i % 4)
    issue_tail(_TAIL[0])

    wait(wuv_v, _S_UV, [r for u in range(4) for r in blk128(u * w_lane + 1, w_lane - 2)])
    ctx = contract(wuv_v)
    own = iota(jnp.int32, (H, H * D), 1) // D == iota(jnp.int32, (H, H * D), 0)
    ctx_bd = jnp.where(own, jnp.concatenate([ctx] * H, axis=1), 0.0).astype(_BF16)
    k2 = H * D // 2
    wait(wo_v, _S_OA, [r for u in (0, 1) for r in blk512(u * w_lane + 1, w_lane - 2)])
    issue_tail(_TAIL[1])
    attn = jnp.sum(_dot(ctx_bd[:, :k2], wo_v[0:k2, :]), axis=0, keepdims=True)
    wait(wo_v, _S_OB, [r for u in (2, 3) for r in blk512(u * w_lane + 1, w_lane - 2)])
    issue_tail(_TAIL[2])
    attn = attn + jnp.sum(_dot(ctx_bd[:, k2:], wo_v[k2:2 * k2, :]), axis=0, keepdims=True)
    x = x + ga * attn

    h2 = (_layernorm(x) * (1.0 + cb) + sb).astype(_BF16)
    assert all(d[2] != _S_D0 for d in tail)
    wait(wd_v, _S_D0, d_fills[0])
    issue_tail(len(tail))
    wait(wg_v, _S_G)
    g = jax.nn.gelu(_dot(h2, wg_v[...]), approximate=True)
    wait(wu_v, _S_U)
    hid = (g * _dot(h2, wu_v[...])).astype(_BF16).astype(_F32)
    eye = iota(jnp.int32, (_LANES, _LANES), 0) == iota(jnp.int32, (_LANES, _LANES), 1)

    def column(lo, hi):
        cols = []
        while lo < hi:
            base = lo // _LANES * _LANES
            end = min(hi, base + _LANES)
            part = jnp.broadcast_to(hid[:, base:base + _LANES], (end - lo, _LANES))
            part = jnp.where(eye[lo - base:end - base], part, 0.0)
            cols.append(jnp.sum(part, axis=1, keepdims=True))
            lo = end
        return cols

    n_d = len(_D_STAGES)
    factor = {}
    for k in range(1, n_d):
        if k < n_d - _D_VPU:
            parts = [hid[:, lo:hi] for lo, hi in d_rows[k]]
            factor[k] = jnp.concatenate(parts, axis=1).astype(_BF16)
        else:
            col = jnp.concatenate([c for lo, hi in d_rows[k] for c in column(lo, hi)], axis=0)
            col = jnp.broadcast_to(col, (col.shape[0], _LANES))
            factor[k] = jnp.concatenate([col] * (M // _LANES), axis=1)
    for k in (n_d - 2, n_d - 1):
        factor[k] = factor[k] * gb
    y = jnp.zeros((8, M), _F32)
    for k in range(1, n_d):
        if k == n_d - 2:
            first_row = iota(jnp.int32, (8, M), 0) == 0
            y = jnp.where(first_row, jnp.broadcast_to(x, (8, M)), 0.0) + gb * y
        wait(wd_v, _S_D0 + k, d_fills[k])
        w = jnp.concatenate([wd_v[lo:hi, :] for lo, hi in d_rows[k]], axis=0)
        if k < n_d - _D_VPU:
            x = x + gb * _dot(factor[k], w)
        else:
            prod = factor[k] * w.astype(_F32)
            for j in range(0, prod.shape[0], 8):
                y = y + prod[j:j + 8]
    x = jnp.sum(y, axis=0, keepdims=True)
    o_ref[...] = x.astype(o_ref.dtype)


def _kernel(*refs, H, D, n_sems):
    pl.run_scoped(
        lambda sems: _body(*refs, sems, H, D), pltpu.SemaphoreType.DMA((n_sems,))
    )


@jax.jit
def pallas_adaLN_cond__compressed_kv_cla__glu_gated_geglu__decode_kernel(
    A_x: jax.Array,
    A_c_kv: jax.Array,
    A_w_q: jax.Array,
    A_w_uk: jax.Array,
    A_w_uv: jax.Array,
    A_w_o: jax.Array,
    B_x: jax.Array,
    B_w_gate: jax.Array,
    B_w_up: jax.Array,
    B_w_down: jax.Array,
    c: jax.Array,
    w_mod: jax.Array,
):
    B, Sq, M = A_x.shape
    Sk, Dc = A_c_kv.shape[1], A_c_kv.shape[2]
    H, D = A_w_q.shape[1], A_w_q.shape[2]
    assert (B, Sq, M, Dc, H, D) == (1, 1, 512, 512, 32, 128) and Sk % 1024 == 0

    operands = (
        A_x.reshape(1, M),
        c,
        w_mod,
        A_w_q.reshape(M * H, D),
        A_w_uk.reshape(Dc * H, D),
        A_c_kv.reshape(Sk, Dc),
        A_w_uv.reshape(Dc * H, D),
        A_w_o.reshape(H * D, M),
        B_w_gate,
        B_w_up,
        B_w_down,
    )
    scratch = [pltpu.VMEM(a.shape, a.dtype) for a in operands]
    scratch += [
        pltpu.VMEM((_LANES, _LANES * H), _BF16),
        pltpu.VMEM((_LANES * H, _LANES), _BF16),
        pltpu.VMEM((4 * H, _LANES * H), _BF16),
    ]
    out = pl.pallas_call(
        functools.partial(_kernel, H=H, D=D, n_sems=_S_KV + Sk // 1024),
        in_specs=[pl.BlockSpec(memory_space=pl.ANY)] * len(operands),
        out_specs=pl.BlockSpec(memory_space=pltpu.VMEM),
        out_shape=jax.ShapeDtypeStruct((1, M), A_x.dtype),
        scratch_shapes=scratch,
        compiler_params=pltpu.CompilerParams(
            vmem_limit_bytes=100 * 1024 * 1024, disable_bounds_checks=True
        ),
    )(*operands)
    return out.reshape(B, Sq, M)
```
